```python
import jax
import jax.numpy as jnp

def _softmax(x, axis=-1):
    return jax.nn.softmax(x, axis=axis)
def _gelu(x):
    return jax.nn.gelu(x, approximate=True)
def _silu(x):
    return jax.nn.silu(x)
def _sigmoid(x):
    return jax.nn.sigmoid(x)
def _layernorm(x, axis=-1, eps=1e-5):
    m = jnp.mean(x, axis=axis, keepdims=True)
    v = jnp.var(x, axis=axis, keepdims=True)
    return (x - m) / jnp.sqrt(v + eps)
def _scatter_add(tgt, idx, src, axis=0):
    return tgt.at[idx].add(src)
def _segment_sum(src, seg, n):
    return jax.ops.segment_sum(src, seg, n)
class _Rng:
    def __init__(self, key):
        self._k = key
    def _next(self):
        self._k, sub = jax.random.split(self._k)
        return sub
    def normal(self, shape):
        return jax.random.normal(self._next(), shape, dtype=jnp.bfloat16)
    def randint(self, lo, hi, shape):
        return jax.random.randint(self._next(), shape, lo, hi, dtype=jnp.int32)
    def uniform(self, shape, lo=0.0, hi=1.0):
        return jax.random.uniform(self._next(), shape, jnp.bfloat16, lo, hi)
    def permutation(self, n):
        return jax.random.permutation(self._next(), n)


kernel_name = 'sequential_preLN__linear_attn_block__moe_arch_mod__prompt'

def setup_inputs():
    _rng = _Rng(jax.random.key(int.from_bytes(__import__("os").urandom(4), "little")))
    _w = (lambda a: (lambda t: t.astype(jnp.bfloat16) if jnp.issubdtype(t.dtype, jnp.floating) else t)(jnp.asarray(a)))
    def _A_setup():
        B, S, D = 1, 2048, 1024
        return {
            "x": _w((lambda *s: _rng.normal(s) * 0.05)(B, S, D)),
            "wqkv": _w((lambda *s: _rng.normal(s) * 0.05)(D, 3 * D)),
            "wo": _w((lambda *s: _rng.normal(s) * 0.05)(D, D)),
        }
    _A_in = _A_setup()

    def _B_setup():
        B, S, D, F, C = 1, 2048, 1024, 3584, 2
        return {
            "x": _w((lambda *s: _rng.normal(s) * 0.05)(B, S, D)),
            "w_r": _w((lambda *s: _rng.normal(s) * 0.05)(D)),
            "w_gate": _w((lambda *s: _rng.normal(s) * 0.05)(D, F)),
            "w_up": _w((lambda *s: _rng.normal(s) * 0.05)(D, F)),
            "w_down": _w((lambda *s: _rng.normal(s) * 0.05)(F, D)),
        }
    _B_in = _B_setup()

    return {
        "A_x": _A_in["x"],
        "A_wqkv": _A_in["wqkv"],
        "A_wo": _A_in["wo"],
        "B_x": _B_in["x"],
        "B_w_r": _B_in["w_r"],
        "B_w_gate": _B_in["w_gate"],
        "B_w_up": _B_in["w_up"],
        "B_w_down": _B_in["w_down"],
    }

def reference(A_x, A_wqkv, A_wo, B_x, B_w_r, B_w_gate, B_w_up, B_w_down):
    def _A_ref(x, wqkv, wo):
        B, S, D = x.shape
        H = 32; Dh = D // H
        qkv = (lambda x, *d: x.transpose(*d))((x @ wqkv).reshape(B, S, 3, H, Dh), 2, 0, 3, 1, 4)
        q, k, v = qkv[0], qkv[1], qkv[2]
        phi = lambda t: jnp.where(t > 0, t + 1, jnp.exp(t)) + 1e-6
        pq, pk = phi(q), phi(k)
        kv = jnp.einsum("bhsd,bhse->bhde", pk, v)
        z = jnp.einsum("bhsd->bhd", pk)
        num = jnp.einsum("bhqd,bhde->bhqe", pq, kv)
        den = jnp.einsum("bhqd,bhd->bhq", pq, z)[..., None] + 1e-6
        o = num / den
        return (lambda x, *d: x.transpose(*d))(o, 0, 2, 1, 3).reshape(B, S, D) @ wo

    def _B_ref(x, w_r, w_gate, w_up, w_down):
        B, S, D = x.shape
        C = 2
        r = x @ w_r
        idx = jnp.argsort(-r, axis=-1)[:, :C]
        idx_e = jnp.repeat(idx.reshape(B, C, 1), D, axis=2)
        x_sel = jnp.take_along_axis(x, idx_e, axis=1)
        g = _silu(x_sel @ w_gate)
        u = x_sel @ w_up
        y = (g * u) @ w_down
        r_sel = _sigmoid(jnp.take_along_axis(r, idx, axis=1))
        y = y * r_sel.reshape(B, C, 1)
        b_off = (jnp.arange(B) * S).reshape(B, 1)
        flat_idx = (idx + b_off).reshape(B * C)
        zero = (x * 0.0).reshape(B * S, D)
        upd = _scatter_add(zero, flat_idx, y.reshape(B * C, D), axis=0)
        return x + upd.reshape(B, S, D)

    x = A_x
    h = x + _A_ref(_layernorm(x, axis=-1), A_wqkv, A_wo)
    h2 = h + _B_ref(_layernorm(h, axis=-1), B_w_r, B_w_gate, B_w_up, B_w_down)
    return h2
```

```python
import functools
import jax
import jax.numpy as jnp
from jax import lax
import jax.experimental.pallas as pl
import jax.experimental.pallas.tpu as pltpu

S, D, F, H, DH = 2048, 1024, 3584, 32, 32
TM = 512
NB = S // TM
NG = D // 128
f32, bf16 = jnp.float32, jnp.bfloat16


def _dot(a, b):
    return jnp.dot(a, b, preferred_element_type=f32)


def _phi(t):
    return jnp.where(t > 0, t + 1.0, jnp.exp(t)) + 1e-6


def _ln(x):
    m = jnp.mean(x, axis=-1, keepdims=True)
    xc = x - m
    v = jnp.mean(xc * xc, axis=-1, keepdims=True)
    return xc * lax.rsqrt(v + 1e-5)


def _kernel(x_hbm, wqkv_hbm, wo_hbm, wr_ref, wg_hbm, wu_hbm, wd_hbm, out_hbm,
            x_v, xn_v, w_v, wo_v, wg_v, wu_v, wd_v, hn_v, out_v, kv_v, z_v, m_v, zbd_v, r_v, fix_v,
            sems):
    c_x0 = pltpu.make_async_copy(x_hbm.at[pl.ds(0, TM)], x_v.at[pl.ds(0, TM)], sems.at[0])
    c_wkv = pltpu.make_async_copy(wqkv_hbm.at[:, pl.ds(D, 2 * D)], w_v.at[:, pl.ds(D, 2 * D)], sems.at[1])
    c_x1 = pltpu.make_async_copy(x_hbm.at[pl.ds(TM, S - TM)], x_v.at[pl.ds(TM, S - TM)], sems.at[2])
    c_wq = pltpu.make_async_copy(wqkv_hbm.at[:, pl.ds(0, D)], w_v.at[:, pl.ds(0, D)], sems.at[3])
    c_wo = pltpu.make_async_copy(wo_hbm, wo_v, sems.at[4])
    c_wg = pltpu.make_async_copy(wg_hbm, wg_v, sems.at[5])
    c_wu = pltpu.make_async_copy(wu_hbm, wu_v, sems.at[6])
    c_wd = pltpu.make_async_copy(wd_hbm, wd_v, sems.at[7])
    c_x0.start()
    c_wkv.start()
    c_x1.start()
    c_wq.start()
    c_wo.start()

    kv_v[...] = jnp.zeros_like(kv_v)
    z_v[...] = jnp.zeros_like(z_v)
    c_x0.wait()
    c_wkv.wait()
    c_wg.start()
    c_wu.start()
    c_wd.start()

    def phase1(b, carry):
        @pl.when(b == 1)
        def _():
            c_x1.wait()
        rows = pl.ds(pl.multiple_of(b * TM, TM), TM)
        xn = _ln(x_v[rows, :].astype(f32)).astype(bf16)
        xn_v[rows, :] = xn
        for j in range(NG):
            k = _dot(xn, w_v[:, D + j * 128:D + (j + 1) * 128])
            v = _dot(xn, w_v[:, 2 * D + j * 128:2 * D + (j + 1) * 128]).astype(bf16)
            pk = _phi(k)
            z_v[:, j * 128:(j + 1) * 128] += pk.reshape(TM // 8, 8, 128).sum(axis=0)
            kv_v[j] += lax.dot_general(pk.astype(bf16), v, (((0,), (0,)), ((), ())),
                                       preferred_element_type=f32)
        return carry

    lax.fori_loop(0, NB, phase1, 0)

    c_wo.wait()
    c_wq.wait()
    ri = lax.broadcasted_iota(jnp.int32, (128, 128), 0) // DH
    ci = lax.broadcasted_iota(jnp.int32, (128, 128), 1) // DH
    bd = ri == ci
    for j in range(NG):
        kvbd = jnp.where(bd, kv_v[j], 0.0).astype(bf16)
        m_v[j * 128:(j + 1) * 128, :] = _dot(kvbd, wo_v[j * 128:(j + 1) * 128, :]).astype(bf16)
        z = jnp.sum(z_v[:, j * 128:(j + 1) * 128], axis=0, keepdims=True)
        zcol = jnp.transpose(jnp.broadcast_to(z, (128, 128)))
        zbd_v[j] = jnp.where(bd, zcol, 0.0).astype(bf16)

    wr = wr_ref[...].astype(f32)

    def phase2(b, carry):
        rows = pl.ds(pl.multiple_of(b * TM, TM), TM)
        xn = xn_v[rows, :]
        parts = []
        for j in range(NG):
            q = _dot(xn, w_v[:, j * 128:(j + 1) * 128])
            pq = _phi(q)
            den = _dot(pq.astype(bf16), zbd_v[j]) + 1e-6
            parts.append((pq / den).astype(bf16))
        pqn = jnp.concatenate(parts, axis=1)
        h = x_v[rows, :].astype(f32) + _dot(pqn, m_v[...])
        hn = _ln(h)
        r = jnp.sum(hn * wr, axis=-1, keepdims=True)
        r_v[rows, :] = jnp.broadcast_to(r, (TM, 128))
        hn_v[rows, :] = hn
        out_v[rows, :] = (h + hn).astype(bf16)
        pltpu.make_async_copy(out_v.at[rows], out_hbm.at[rows], sems.at[8 + b]).start()
        return carry

    lax.fori_loop(0, NB, phase2, 0)

    r = r_v[...]
    io = lax.broadcasted_iota(jnp.int32, (S, 128), 0)
    m1 = jnp.max(r)
    i1 = jnp.min(jnp.where(r == m1, io, S))
    r2 = jnp.where(io == i1, -jnp.inf, r)
    m2 = jnp.max(r2)
    i2 = jnp.min(jnp.where(r2 == m2, io, S))

    b1 = pl.multiple_of((i1 // 16) * 16, 16)
    b2 = pl.multiple_of((i2 // 16) * 16, 16)
    io16 = lax.broadcasted_iota(jnp.int32, (16, D), 0)
    s1 = jnp.sum(jnp.where(io16 == i1 - b1, hn_v[pl.ds(b1, 16), :], 0.0), axis=0, keepdims=True)
    s2 = jnp.sum(jnp.where(io16 == i2 - b2, hn_v[pl.ds(b2, 16), :], 0.0), axis=0, keepdims=True)
    io8 = lax.broadcasted_iota(jnp.int32, (16, D), 0)
    xs = jnp.where(io8 == 0, s1, jnp.where(io8 == 1, s2, 0.0)).astype(bf16)
    c_wg.wait()
    c_wu.wait()
    c_wd.wait()
    g = _dot(xs, wg_v[...])
    u = _dot(xs, wu_v[...])
    a = (g * jax.nn.sigmoid(g) * u).astype(bf16)
    y = _dot(a, wd_v[...])
    y1 = y[0:1, :] * jax.nn.sigmoid(jnp.full((1, D), m1, f32))
    y2 = y[1:2, :] * jax.nn.sigmoid(jnp.full((1, D), m2, f32))

    for b in range(NB):
        rows = pl.ds(b * TM, TM)
        pltpu.make_async_copy(out_v.at[rows], out_hbm.at[rows], sems.at[8 + b]).wait()

    o1 = out_v[pl.ds(b1, 16), :].astype(f32) + jnp.where(io16 == i1 - b1, y1, 0.0)
    out_v[pl.ds(b1, 16), :] = o1.astype(bf16)
    o2 = out_v[pl.ds(b2, 16), :].astype(f32) + jnp.where(io16 == i2 - b2, y2, 0.0)
    out_v[pl.ds(b2, 16), :] = o2.astype(bf16)
    f1 = pltpu.make_async_copy(out_v.at[pl.ds(b1, 16)], out_hbm.at[pl.ds(b1, 16)], sems.at[8])
    f1.start()
    f1.wait()
    f2 = pltpu.make_async_copy(out_v.at[pl.ds(b2, 16)], out_hbm.at[pl.ds(b2, 16)], sems.at[9])
    f2.start()
    f2.wait()


@jax.jit
def pallas_sequential_preLN__linear_attn_block__moe_arch_mod__prompt_kernel(
    A_x, A_wqkv, A_wo, B_x, B_w_r, B_w_gate, B_w_up, B_w_down,
):
    del B_x
    any_spec = pl.BlockSpec(memory_space=pl.ANY)
    out = pl.pallas_call(
        _kernel,
        in_specs=[any_spec, any_spec, any_spec, pl.BlockSpec(memory_space=pltpu.VMEM),
                  any_spec, any_spec, any_spec],
        out_specs=any_spec,
        out_shape=jax.ShapeDtypeStruct((S, D), bf16),
        scratch_shapes=[
            pltpu.VMEM((S, D), bf16),
            pltpu.VMEM((S, D), bf16),
            pltpu.VMEM((D, 3 * D), bf16),
            pltpu.VMEM((D, D), bf16),
            pltpu.VMEM((D, F), bf16),
            pltpu.VMEM((D, F), bf16),
            pltpu.VMEM((F, D), bf16),
            pltpu.VMEM((S, D), f32),
            pltpu.VMEM((S, D), bf16),
            pltpu.VMEM((NG, 128, 128), f32),
            pltpu.VMEM((8, D), f32),
            pltpu.VMEM((D, D), bf16),
            pltpu.VMEM((NG, 128, 128), bf16),
            pltpu.VMEM((S, 128), f32),
            pltpu.VMEM((16, D), bf16),
            pltpu.SemaphoreType.DMA((16,)),
        ],
        compiler_params=pltpu.CompilerParams(vmem_limit_bytes=100 * 1024 * 1024),
    )(A_x.reshape(S, D), A_wqkv, A_wo, B_w_r.reshape(1, D), B_w_gate, B_w_up, B_w_down)
    return out.reshape(1, S, D)
```

```python
import functools
import jax
import jax.numpy as jnp
from jax import lax
import jax.experimental.pallas as pl
import jax.experimental.pallas.tpu as pltpu

S, D, F, H, DH = 2048, 1024, 3584, 32, 32
TM = 512
NB = S // TM
NG = D // 128
CW = 512
NC = D // CW
LATE = 0
PR = 32
CW2 = 256
f32, bf16 = jnp.float32, jnp.bfloat16
_TN = (((0,), (0,)), ((), ()))


def _dot(a, b):
    return jnp.dot(a, b, preferred_element_type=f32)


def _phi(t):
    return jnp.where(t > 0, t + 1.0, jnp.exp(t)) + 1e-6


def _ln(x):
    m = jnp.mean(x, axis=-1, keepdims=True)
    xc = x - m
    v = jnp.mean(xc * xc, axis=-1, keepdims=True)
    return xc * lax.rsqrt(v + 1e-5)


def _kernel(x_hbm, wqkv_hbm, wo_hbm, wr_ref, wg_hbm, wu_hbm, wd_hbm, out_hbm,
            x_v, xn_v, w_v, wo_v, wg_v, wu_v, wd_v, h_v, out_v, kv_v, z_v, m_v, zbd_v, fix_v, pqn_v,
            sems):
    nsem = [0]

    def copy(src, dst):
        c = pltpu.make_async_copy(src, dst, sems.at[nsem[0]])
        nsem[0] += 1
        return c

    def wcopy(c0, n):
        return copy(wqkv_hbm.at[:, pl.ds(c0, n)], w_v.at[:, pl.ds(c0, n)])

    c_x = [copy(x_hbm.at[pl.ds(b * TM, TM)], x_v.at[pl.ds(b * TM, TM)]) for b in range(NB)]
    c_k = [wcopy(D + j * CW, CW) for j in range(NC)]
    c_v = [wcopy(2 * D + j * CW, CW) for j in range(NC)]
    c_q = wcopy(0, D)
    c_wo = copy(wo_hbm, wo_v)
    fsem = nsem[0]
    nsem[0] += 3
    c_ffn = []
    for t, (src, dst) in enumerate([(wg_hbm, wg_v), (wu_hbm, wu_v), (wd_hbm, wd_v)]):
        for j in range(dst.shape[0]):
            c_ffn.append(pltpu.make_async_copy(src.at[:, pl.ds(j * 128, 128)], dst.at[j], sems.at[fsem + t]))
    c_out = [copy(out_v.at[pl.ds(b * TM, TM)], out_hbm.at[pl.ds(b * TM, TM)]) for b in range(NB)]
    fix_sems = [sems.at[nsem[0]], sems.at[nsem[0] + 1]]

    for c in [c_x[0], c_k[0], c_v[0], c_k[1], c_x[1], c_v[1], c_x[2], c_x[3], c_q, c_wo] + c_ffn:
        c.start()

    def ln_x(r0, n):
        xn_v[r0:r0 + n, :] = _ln(x_v[r0:r0 + n, :].astype(f32)).astype(bf16)

    c_x[0].wait()
    ln_x(0, TM)

    for b in range(NB):
        rows = slice(b * TM, (b + 1) * TM)
        nxt = [(b + 1) * TM + i * (TM // 4) for i in range(4)] if b + 1 < NB else []
        step = 0
        for j in range(NC):
            cs = slice(j * CW, (j + 1) * CW)
            if b == 0:
                c_k[j].wait()
            k = _dot(xn_v[rows, :], w_v[:, D + j * CW:D + (j + 1) * CW])
            if nxt and step == 0 and b > 0:
                c_x[b + 1].wait()
            if b == 0 and j == 1:
                c_x[1].wait()
            pk = _phi(k)
            zs = pk.reshape(TM // 8, 8, CW).sum(axis=0)
            if b == 0:
                z_v[:, cs] = zs
            else:
                z_v[:, cs] += zs
            pk = pk.astype(bf16)
            if nxt and (b > 0 or j == 1):
                if b == 0:
                    ln_x(nxt[0], TM // 2)
                else:
                    ln_x(nxt[step], TM // 4)
            step += 1
            if b == 0:
                c_v[j].wait()
            v = _dot(xn_v[rows, :], w_v[:, 2 * D + j * CW:2 * D + (j + 1) * CW]).astype(bf16)
            if nxt and (b > 0 or j == 1):
                if b == 0:
                    ln_x(nxt[2], TM // 2)
                else:
                    ln_x(nxt[step], TM // 4)
            step += 1
            for i in range(CW // 128):
                g = j * (CW // 128) + i
                kv = lax.dot_general(pk[:, i * 128:(i + 1) * 128], v[:, i * 128:(i + 1) * 128], _TN,
                                     preferred_element_type=f32)
                if b == 0:
                    kv_v[g] = kv
                else:
                    kv_v[g] += kv

    c_wo.wait()
    c_q.wait()
    ri = lax.broadcasted_iota(jnp.int32, (128, 128), 0) // DH
    ci = lax.broadcasted_iota(jnp.int32, (128, 128), 1) // DH
    bd = ri == ci
    for j in range(NG):
        kvbd = jnp.where(bd, kv_v[j], 0.0).astype(bf16)
        m_v[j * 128:(j + 1) * 128, :] = _dot(kvbd, wo_v[j * 128:(j + 1) * 128, :]).astype(bf16)
        z = jnp.sum(z_v[:, j * 128:(j + 1) * 128], axis=0, keepdims=True)
        zcol = jnp.transpose(jnp.broadcast_to(z, (128, 128)))
        zbd_v[j] = jnp.where(bd, zcol, 0.0).astype(bf16)

    wr = wr_ref[...].astype(f32).reshape(1, D)
    lane3 = lax.broadcasted_iota(jnp.int32, (PR // 8, 8, 128), 2)
    t3 = lax.broadcasted_iota(jnp.int32, (PR // 8, 8, 128), 0)
    rd = [jnp.full((8, 128), -jnp.inf, f32) for _ in range(S // 1024)]

    def post(r0, n):
        h = h_v[r0:r0 + n, :]
        hn = _ln(h)
        r = jnp.sum(hn * wr, axis=-1, keepdims=True)
        r3 = jnp.broadcast_to(r, (n, 128)).reshape(n // 8, 8, 128)
        sel = jnp.where(lane3 == t3 + (r0 // 8) % 128, r3, -jnp.inf).max(axis=0)
        rd[r0 // 1024] = jnp.maximum(rd[r0 // 1024], sel)
        out_v[r0:r0 + n, :] = (h + hn).astype(bf16)

    def qstage(b, j):
        rows = slice(b * TM, (b + 1) * TM)
        q = _dot(xn_v[rows, :], w_v[:, j * CW2:(j + 1) * CW2])
        pq = _phi(q)
        pqb = pq.astype(bf16)
        den = jnp.concatenate(
            [_dot(pqb[:, i * 128:(i + 1) * 128], zbd_v[j * (CW2 // 128) + i]) for i in range(CW2 // 128)],
            axis=1) + 1e-6
        pqn_v[rows, j * CW2:(j + 1) * CW2] = (pq * pltpu.reciprocal(den, approx=True)).astype(bf16)

    def ostage(b, j):
        rows = slice(b * TM, (b + 1) * TM)
        cs = slice(j * CW2, (j + 1) * CW2)
        h_v[rows, cs] = x_v[rows, cs].astype(f32) + _dot(pqn_v[rows, :], m_v[:, cs])

    NC2 = D // CW2
    pending = []
    for b in range(NB + 1):
        for j in range(NC2):
            if b < NB:
                qstage(b, j)
            npc = TM // PR // NC2 // 2
            for _ in range(npc):
                if pending:
                    post(pending.pop(0), PR)
            if b > 0:
                ostage(b - 1, j)
            for _ in range(npc):
                if pending:
                    post(pending.pop(0), PR)
        if b > 1 and not LATE:
            c_out[b - 2].start()
        if b > 0:
            pending = [(b - 1) * TM + i * PR for i in range(TM // PR)]
    for r0 in pending:
        post(r0, PR)
    if LATE:
        for c in c_out[:-1]:
            c.start()
    c_out[NB - 1].start()

    idx = [lax.broadcasted_iota(jnp.int32, (8, 128), 1) * 8 + lax.broadcasted_iota(jnp.int32, (8, 128), 0)
           + t * 1024 for t in range(S // 1024)]

    def top1(vals):
        mx = functools.reduce(jnp.maximum, vals)
        mx = jnp.max(jnp.max(mx, axis=1, keepdims=True), axis=0, keepdims=True)
        cand = functools.reduce(jnp.minimum, [jnp.where(v == mx, i, S) for v, i in zip(vals, idx)])
        ix = jnp.min(jnp.min(cand, axis=1, keepdims=True), axis=0, keepdims=True)
        return mx, ix

    m1, i1v = top1(rd)
    rd2 = [jnp.where(i == i1v, -jnp.inf, v) for v, i in zip(rd, idx)]
    m2, i2v = top1(rd2)
    i1 = jnp.clip(i1v[0, 0], 0, S - 1)
    i2 = jnp.clip(i2v[0, 0], 0, S - 1)

    b1 = pl.multiple_of((i1 // 16) * 16, 16)
    b2 = pl.multiple_of((i2 // 16) * 16, 16)
    io16 = lax.broadcasted_iota(jnp.int32, (16, D), 0)
    s1 = jnp.sum(jnp.where(io16 == i1 - b1, _ln(h_v[pl.ds(b1, 16), :]), 0.0), axis=0, keepdims=True)
    s2 = jnp.sum(jnp.where(io16 == i2 - b2, _ln(h_v[pl.ds(b2, 16), :]), 0.0), axis=0, keepdims=True)
    xs = jnp.where(io16 == 0, s1, jnp.where(io16 == 1, s2, 0.0)).astype(bf16)
    for c in c_ffn:
        c.wait()
    cat = lambda ref: jnp.concatenate([ref[j] for j in range(ref.shape[0])], axis=1)
    g = _dot(xs, cat(wg_v))
    u = _dot(xs, cat(wu_v))
    a = (g * jax.nn.sigmoid(g) * u).astype(bf16)
    y = _dot(a, cat(wd_v))
    y1 = y[0:1, :] * jax.nn.sigmoid(m1)
    y2 = y[1:2, :] * jax.nn.sigmoid(m2)

    o1 = (out_v[pl.ds(b1, 16), :].astype(f32) + jnp.where(io16 + b1 == i1, y1, 0.0)
          + jnp.where(io16 + b1 == i2, y2, 0.0))
    o2 = out_v[pl.ds(b2, 16), :].astype(f32) + jnp.where(io16 + b2 == i2, y2, 0.0)
    fix_v[0] = o1.astype(bf16)
    fix_v[1] = o2.astype(bf16)
    for c in c_out:
        c.wait()
    f1 = pltpu.make_async_copy(fix_v.at[0], out_hbm.at[pl.ds(b1, 16)], fix_sems[0])
    f2 = pltpu.make_async_copy(fix_v.at[1], out_hbm.at[pl.ds(b2, 16)], fix_sems[1])
    f1.start()

    @pl.when(b1 != b2)
    def _():
        f2.start()
        f2.wait()

    f1.wait()


@jax.jit
def pallas_sequential_preLN__linear_attn_block__moe_arch_mod__prompt_kernel(
    A_x, A_wqkv, A_wo, B_x, B_w_r, B_w_gate, B_w_up, B_w_down,
):
    del B_x
    any_spec = pl.BlockSpec(memory_space=pl.ANY)
    out = pl.pallas_call(
        _kernel,
        in_specs=[any_spec, any_spec, any_spec, pl.BlockSpec(memory_space=pltpu.VMEM),
                  any_spec, any_spec, any_spec],
        out_specs=any_spec,
        out_shape=jax.ShapeDtypeStruct((S, D), bf16),
        scratch_shapes=[
            pltpu.VMEM((S, D), bf16),
            pltpu.VMEM((S, D), bf16),
            pltpu.VMEM((D, 3 * D), bf16),
            pltpu.VMEM((D, D), bf16),
            pltpu.VMEM((F // 128, D, 128), bf16),
            pltpu.VMEM((F // 128, D, 128), bf16),
            pltpu.VMEM((D // 128, F, 128), bf16),
            pltpu.VMEM((S, D), f32),
            pltpu.VMEM((S, D), bf16),
            pltpu.VMEM((NG, 128, 128), f32),
            pltpu.VMEM((8, D), f32),
            pltpu.VMEM((D, D), bf16),
            pltpu.VMEM((NG, 128, 128), bf16),
            pltpu.VMEM((2, 16, D), bf16),
            pltpu.VMEM((S, D), bf16),
            pltpu.SemaphoreType.DMA((24,)),
        ],
        compiler_params=pltpu.CompilerParams(vmem_limit_bytes=100 * 1024 * 1024, flags={'XLA_TPU_EVENLY_DISTRIBUTE_CRITICAL_NODES': True}),
    )(A_x.reshape(S, D), A_wqkv, A_wo, B_w_r, B_w_gate, B_w_up, B_w_down)
    return out.reshape(1, S, D)
```

```python
import functools
import jax
import jax.numpy as jnp
from jax import lax
import jax.experimental.pallas as pl
import jax.experimental.pallas.tpu as pltpu

S, D, F, H, DH = 2048, 1024, 3584, 32, 32
TM = 512
NB = S // TM
NG = D // 128
CW = 512
NC = D // CW
LATE = 0
PR = 32
CW2 = 256
f32, bf16 = jnp.float32, jnp.bfloat16
_TN = (((0,), (0,)), ((), ()))


def _dot(a, b):
    return jnp.dot(a, b, preferred_element_type=f32)


def _phi(t):
    return jnp.where(t > 0, t + 1.0, jnp.exp(t)) + 1e-6


def _ln(x):
    m = jnp.mean(x, axis=-1, keepdims=True)
    xc = x - m
    v = jnp.mean(xc * xc, axis=-1, keepdims=True)
    return xc * lax.rsqrt(v + 1e-5)


def _kernel(x_hbm, wqkv_hbm, wo_hbm, wr_ref, wg_hbm, wu_hbm, wd_hbm, out_hbm,
            x_v, xn_v, w_v, wo_v, wg_v, wu_v, wd_v, h_v, out_v, kv_v, z_v, m_v, zbd_v, fix_v, pqn_v,
            sems):
    nsem = [0]

    def copy(src, dst):
        c = pltpu.make_async_copy(src, dst, sems.at[nsem[0]])
        nsem[0] += 1
        return c

    def wcopy(c0, n):
        return copy(wqkv_hbm.at[:, pl.ds(c0, n)], w_v.at[:, pl.ds(c0, n)])

    c_x = [copy(x_hbm.at[pl.ds(b * TM, TM)], x_v.at[pl.ds(b * TM, TM)]) for b in range(NB)]
    c_k = [wcopy(D + j * CW, CW) for j in range(NC)]
    c_v = [wcopy(2 * D + j * CW, CW) for j in range(NC)]
    c_q = wcopy(0, D)
    c_wo = copy(wo_hbm, wo_v)
    fsem = nsem[0]
    nsem[0] += 3
    c_ffn = []
    for t, (src, dst) in enumerate([(wg_hbm, wg_v), (wu_hbm, wu_v), (wd_hbm, wd_v)]):
        for j in range(dst.shape[0]):
            c_ffn.append(pltpu.make_async_copy(src.at[:, pl.ds(j * 128, 128)], dst.at[j], sems.at[fsem + t]))
    c_out = [copy(out_v.at[pl.ds(b * TM, TM)], out_hbm.at[pl.ds(b * TM, TM)]) for b in range(NB)]
    fix_sems = [sems.at[nsem[0]], sems.at[nsem[0] + 1]]

    for c in [c_x[0], c_k[0], c_v[0], c_k[1], c_x[1], c_v[1], c_x[2], c_x[3], c_q, c_wo] + c_ffn:
        c.start()

    def ln_x(r0, n):
        xn_v[r0:r0 + n, :] = _ln(x_v[r0:r0 + n, :].astype(f32)).astype(bf16)

    c_x[0].wait()
    ln_x(0, TM)

    for b in range(NB):
        rows = slice(b * TM, (b + 1) * TM)
        nxt = [(b + 1) * TM + i * (TM // 4) for i in range(4)] if b + 1 < NB else []
        step = 0
        for j in range(NC):
            cs = slice(j * CW, (j + 1) * CW)
            if b == 0:
                c_k[j].wait()
            k = _dot(xn_v[rows, :], w_v[:, D + j * CW:D + (j + 1) * CW])
            if nxt and step == 0 and b > 0:
                c_x[b + 1].wait()
            if b == 0 and j == 1:
                c_x[1].wait()
            pk = _phi(k)
            zs = pk.reshape(TM // 8, 8, CW).sum(axis=0)
            if b == 0:
                z_v[:, cs] = zs
            else:
                z_v[:, cs] += zs
            pk = pk.astype(bf16)
            if nxt and (b > 0 or j == 1):
                if b == 0:
                    ln_x(nxt[0], TM // 2)
                else:
                    ln_x(nxt[step], TM // 4)
            step += 1
            if b == 0:
                c_v[j].wait()
            v = _dot(xn_v[rows, :], w_v[:, 2 * D + j * CW:2 * D + (j + 1) * CW]).astype(bf16)
            if nxt and (b > 0 or j == 1):
                if b == 0:
                    ln_x(nxt[2], TM // 2)
                else:
                    ln_x(nxt[step], TM // 4)
            step += 1
            for i in range(CW // 128):
                g = j * (CW // 128) + i
                kv = lax.dot_general(pk[:, i * 128:(i + 1) * 128], v[:, i * 128:(i + 1) * 128], _TN,
                                     preferred_element_type=f32)
                if b == 0:
                    kv_v[g] = kv
                else:
                    kv_v[g] += kv

    c_wo.wait()
    c_q.wait()
    ri = lax.broadcasted_iota(jnp.int32, (128, 128), 0) // DH
    ci = lax.broadcasted_iota(jnp.int32, (128, 128), 1) // DH
    bd = ri == ci
    for j in range(NG):
        kvbd = jnp.where(bd, kv_v[j], 0.0).astype(bf16)
        m_v[j * 128:(j + 1) * 128, :] = _dot(kvbd, wo_v[j * 128:(j + 1) * 128, :]).astype(bf16)
        z = jnp.sum(z_v[:, j * 128:(j + 1) * 128], axis=0, keepdims=True)
        zcol = jnp.transpose(jnp.broadcast_to(z, (128, 128)))
        zbd_v[j] = jnp.where(bd, zcol, 0.0).astype(bf16)

    wr = wr_ref[...].astype(f32).reshape(1, D)
    lane3 = lax.broadcasted_iota(jnp.int32, (PR // 8, 8, 128), 2)
    t3 = lax.broadcasted_iota(jnp.int32, (PR // 8, 8, 128), 0)
    rd = [jnp.full((8, 128), -jnp.inf, f32) for _ in range(S // 1024)]

    def post(r0, n):
        h = h_v[r0:r0 + n, :]
        hn = _ln(h)
        r = jnp.sum(hn * wr, axis=-1, keepdims=True)
        r3 = jnp.broadcast_to(r, (n, 128)).reshape(n // 8, 8, 128)
        sel = jnp.where(lane3 == t3 + (r0 // 8) % 128, r3, -jnp.inf).max(axis=0)
        rd[r0 // 1024] = jnp.maximum(rd[r0 // 1024], sel)
        out_v[r0:r0 + n, :] = (h + hn).astype(bf16)

    def qstage(b, j):
        rows = slice(b * TM, (b + 1) * TM)
        q = _dot(xn_v[rows, :], w_v[:, j * CW2:(j + 1) * CW2])
        pq = _phi(q)
        pqb = pq.astype(bf16)
        den = jnp.concatenate(
            [_dot(pqb[:, i * 128:(i + 1) * 128], zbd_v[j * (CW2 // 128) + i]) for i in range(CW2 // 128)],
            axis=1) + 1e-6
        pqn_v[rows, j * CW2:(j + 1) * CW2] = (pq * pltpu.reciprocal(den, approx=True)).astype(bf16)

    def ostage(b, j):
        n = TM // (D // CW2)
        rows = slice(b * TM + j * n, b * TM + (j + 1) * n)
        h_v[rows, :] = x_v[rows, :].astype(f32) + _dot(pqn_v[rows, :], m_v[...])

    NC2 = D // CW2
    pending = []
    for b in range(NB + 1):
        if b == NB:
            n = TM // 4
            for i in range(4):
                rows = slice(S - TM + i * n, S - TM + (i + 1) * n)
                for _ in range(n // PR):
                    post(pending.pop(0), PR)
                h_v[rows, :] = x_v[rows, :].astype(f32) + _dot(pqn_v[rows, :], m_v[...])
            c_out[b - 2].start()
            pending = [S - TM + i * PR for i in range(TM // PR)]
            break
        for j in range(NC2):
            if b < NB:
                qstage(b, j)
            npc = TM // PR // NC2 // 2
            for _ in range(npc):
                if pending:
                    post(pending.pop(0), PR)
            if b > 0:
                ostage(b - 1, j)
            for _ in range(npc):
                if pending:
                    post(pending.pop(0), PR)
        if b > 1 and not LATE:
            c_out[b - 2].start()
        if b > 0:
            pending = [(b - 1) * TM + i * PR for i in range(TM // PR)]
    for r0 in pending:
        post(r0, PR)
    if LATE:
        for c in c_out[:-1]:
            c.start()
    c_out[NB - 1].start()

    idx = [lax.broadcasted_iota(jnp.int32, (8, 128), 1) * 8 + lax.broadcasted_iota(jnp.int32, (8, 128), 0)
           + t * 1024 for t in range(S // 1024)]

    def top1(vals):
        mx = functools.reduce(jnp.maximum, vals)
        mx = jnp.max(jnp.max(mx, axis=1, keepdims=True), axis=0, keepdims=True)
        cand = functools.reduce(jnp.minimum, [jnp.where(v == mx, i, S) for v, i in zip(vals, idx)])
        ix = jnp.min(jnp.min(cand, axis=1, keepdims=True), axis=0, keepdims=True)
        return mx, ix

    m1, i1v = top1(rd)
    rd2 = [jnp.where(i == i1v, -jnp.inf, v) for v, i in zip(rd, idx)]
    m2, i2v = top1(rd2)
    i1 = jnp.clip(i1v[0, 0], 0, S - 1)
    i2 = jnp.clip(i2v[0, 0], 0, S - 1)

    b1 = pl.multiple_of((i1 // 16) * 16, 16)
    b2 = pl.multiple_of((i2 // 16) * 16, 16)
    io16 = lax.broadcasted_iota(jnp.int32, (16, D), 0)
    s1 = jnp.sum(jnp.where(io16 == i1 - b1, _ln(h_v[pl.ds(b1, 16), :]), 0.0), axis=0, keepdims=True)
    s2 = jnp.sum(jnp.where(io16 == i2 - b2, _ln(h_v[pl.ds(b2, 16), :]), 0.0), axis=0, keepdims=True)
    xs = jnp.where(io16 == 0, s1, jnp.where(io16 == 1, s2, 0.0)).astype(bf16)
    for c in c_ffn:
        c.wait()
    cat = lambda ref: jnp.concatenate([ref[j] for j in range(ref.shape[0])], axis=1)
    g = _dot(xs, cat(wg_v))
    u = _dot(xs, cat(wu_v))
    a = (g * jax.nn.sigmoid(g) * u).astype(bf16)
    y = _dot(a, cat(wd_v))
    y1 = y[0:1, :] * jax.nn.sigmoid(m1)
    y2 = y[1:2, :] * jax.nn.sigmoid(m2)

    o1 = (out_v[pl.ds(b1, 16), :].astype(f32) + jnp.where(io16 + b1 == i1, y1, 0.0)
          + jnp.where(io16 + b1 == i2, y2, 0.0))
    o2 = out_v[pl.ds(b2, 16), :].astype(f32) + jnp.where(io16 + b2 == i2, y2, 0.0)
    fix_v[0] = o1.astype(bf16)
    fix_v[1] = o2.astype(bf16)
    for c in c_out:
        c.wait()
    f1 = pltpu.make_async_copy(fix_v.at[0], out_hbm.at[pl.ds(b1, 16)], fix_sems[0])
    f2 = pltpu.make_async_copy(fix_v.at[1], out_hbm.at[pl.ds(b2, 16)], fix_sems[1])
    f1.start()

    @pl.when(b1 != b2)
    def _():
        f2.start()
        f2.wait()

    f1.wait()


@jax.jit
def pallas_sequential_preLN__linear_attn_block__moe_arch_mod__prompt_kernel(
    A_x, A_wqkv, A_wo, B_x, B_w_r, B_w_gate, B_w_up, B_w_down,
):
    del B_x
    any_spec = pl.BlockSpec(memory_space=pl.ANY)
    out = pl.pallas_call(
        _kernel,
        in_specs=[any_spec, any_spec, any_spec, pl.BlockSpec(memory_space=pltpu.VMEM),
                  any_spec, any_spec, any_spec],
        out_specs=any_spec,
        out_shape=jax.ShapeDtypeStruct((S, D), bf16),
        scratch_shapes=[
            pltpu.VMEM((S, D), bf16),
            pltpu.VMEM((S, D), bf16),
            pltpu.VMEM((D, 3 * D), bf16),
            pltpu.VMEM((D, D), bf16),
            pltpu.VMEM((F // 128, D, 128), bf16),
            pltpu.VMEM((F // 128, D, 128), bf16),
            pltpu.VMEM((D // 128, F, 128), bf16),
            pltpu.VMEM((S, D), f32),
            pltpu.VMEM((S, D), bf16),
            pltpu.VMEM((NG, 128, 128), f32),
            pltpu.VMEM((8, D), f32),
            pltpu.VMEM((D, D), bf16),
            pltpu.VMEM((NG, 128, 128), bf16),
            pltpu.VMEM((2, 16, D), bf16),
            pltpu.VMEM((S, D), bf16),
            pltpu.SemaphoreType.DMA((24,)),
        ],
        compiler_params=pltpu.CompilerParams(vmem_limit_bytes=100 * 1024 * 1024, flags={'XLA_TPU_EVENLY_DISTRIBUTE_CRITICAL_NODES': True}),
    )(A_x.reshape(S, D), A_wqkv, A_wo, B_w_r, B_w_gate, B_w_up, B_w_down)
    return out.reshape(1, S, D)
```
